```python
import jax
import jax.numpy as jnp

def _softmax(x, axis=-1):
    return jax.nn.softmax(x, axis=axis)

def _gelu(x):
    return jax.nn.gelu(x, approximate=True)

def _silu(x):
    return jax.nn.silu(x)

def _sigmoid(x):
    return jax.nn.sigmoid(x)

def _layernorm(x, axis=-1, eps=1e-05):
    m = jnp.mean(x, axis=axis, keepdims=True)
    v = jnp.var(x, axis=axis, keepdims=True)
    return (x - m) / jnp.sqrt(v + eps)

def _scatter_add(tgt, idx, src, axis=0):
    return tgt.at[idx].add(src)

def _segment_sum(src, seg, n):
    return jax.ops.segment_sum(src, seg, n)

class _Rng:

    def __init__(self, key):
        self._k = key

    def _next(self):
        self._k, sub = jax.random.split(self._k)
        return sub

    def normal(self, shape):
        return jax.random.normal(self._next(), shape, dtype=jnp.bfloat16)

    def randint(self, lo, hi, shape):
        return jax.random.randint(self._next(), shape, lo, hi, dtype=jnp.int32)

    def uniform(self, shape, lo=0.0, hi=1.0):
        return jax.random.uniform(self._next(), shape, jnp.bfloat16, lo, hi)

    def permutation(self, n):
        return jax.random.permutation(self._next(), n)
kernel_name = 'adaLN_cond__mha_block_cached__moe_arch_mod__decode'

def setup_inputs():
    _rng = _Rng(jax.random.key(int.from_bytes(__import__("os").urandom(4), "little")))
    _w = lambda a: (lambda t: t.astype(jnp.bfloat16) if jnp.issubdtype(t.dtype, jnp.floating) else t)(jnp.asarray(a))

    def _A_setup():
        B, Sq, D = (4, 1, 448)
        H, Sk, Dh = (16, 16384, 256)
        return {'x': _w((lambda *s: _rng.normal(s) * 0.05)(B, Sq, D)), 'k_cache': _w((lambda *s: _rng.normal(s) * 0.05)(B, H, Sk, Dh)), 'v_cache': _w((lambda *s: _rng.normal(s) * 0.05)(B, H, Sk, Dh)), 'wq': _w((lambda *s: _rng.normal(s) * 0.05)(D, H * Dh) * D ** (-0.5)), 'wo': _w((lambda *s: _rng.normal(s) * 0.05)(H * Dh, D) * (H * Dh) ** (-0.5))}
    _A_in = _A_setup()

    def _B_setup():
        B, S, D, F, C = (4, 1, 448, 1792, 1)
        return {'x': _w((lambda *s: _rng.normal(s) * 0.05)(B, S, D)), 'w_r': _w((lambda *s: _rng.normal(s) * 0.05)(D)), 'w_gate': _w((lambda *s: _rng.normal(s) * 0.05)(D, F)), 'w_up': _w((lambda *s: _rng.normal(s) * 0.05)(D, F)), 'w_down': _w((lambda *s: _rng.normal(s) * 0.05)(F, D))}
    _B_in = _B_setup()
    return {'A_x': _A_in['x'], 'A_k_cache': _A_in['k_cache'], 'A_v_cache': _A_in['v_cache'], 'A_wq': _A_in['wq'], 'A_wo': _A_in['wo'], 'B_x': _B_in['x'], 'B_w_r': _B_in['w_r'], 'B_w_gate': _B_in['w_gate'], 'B_w_up': _B_in['w_up'], 'B_w_down': _B_in['w_down'], 'c': _w((lambda *s: _rng.normal(s) * 0.05)(4, 448)), 'w_mod': _w((lambda *s: _rng.normal(s) * 0.05)(448, 6 * 448) * 448 ** (-0.5))}

def reference(A_x, A_k_cache, A_v_cache, A_wq, A_wo, B_x, B_w_r, B_w_gate, B_w_up, B_w_down, c, w_mod):

    def _A_ref(x, k_cache, v_cache, wq, wo):
        B, Sq, D = x.shape
        H, Dh = (16, 256)
        q = (lambda x, *d: x.transpose(*d))((x @ wq).reshape(B, Sq, H, Dh), 0, 2, 1, 3)
        scores = jnp.einsum('bhqd,bhkd->bhqk', q, k_cache) * Dh ** (-0.5)
        p = _softmax(scores, axis=-1)
        o = jnp.einsum('bhqk,bhkd->bhqd', p, v_cache)
        return (lambda x, *d: x.transpose(*d))(o, 0, 2, 1, 3).reshape(B, Sq, H * Dh) @ wo

    def _B_ref(x, w_r, w_gate, w_up, w_down):
        B, S, D = x.shape
        C = 1
        r = x @ w_r
        idx = jnp.argsort(-r, axis=-1)[:, :C]
        idx_e = jnp.repeat(idx.reshape(B, C, 1), D, axis=2)
        x_sel = jnp.take_along_axis(x, idx_e, axis=1)
        g = _silu(x_sel @ w_gate)
        u = x_sel @ w_up
        y = g * u @ w_down
        r_sel = _sigmoid(jnp.take_along_axis(r, idx, axis=1))
        y = y * r_sel.reshape(B, C, 1)
        b_off = (jnp.arange(B) * S).reshape(B, 1)
        flat_idx = (idx + b_off).reshape(B * C)
        zero = (x * 0.0).reshape(B * S, D)
        upd = _scatter_add(zero, flat_idx, y.reshape(B * C, D), axis=0)
        return x + upd.reshape(B, S, D)
    x = A_x
    mod = (_silu(c) @ w_mod).reshape(c.shape[0], 6, 1, -1)
    sa, ca, ga, sb, cb, gb = (mod[:, 0].copy(), mod[:, 1].copy(), mod[:, 2].copy(), mod[:, 3].copy(), mod[:, 4].copy(), mod[:, 5].copy())
    h = _layernorm(x, axis=-1) * (1 + ca) + sa
    x = x + ga * _A_ref(h, A_k_cache, A_v_cache, A_wq, A_wo)
    h = _layernorm(x, axis=-1) * (1 + cb) + sb
    x = x + gb * _B_ref(h, B_w_r, B_w_gate, B_w_up, B_w_down)
    return x
```

```python
import jax
import jax.numpy as jnp
from jax import lax
import jax.experimental.pallas as pl
import jax.experimental.pallas.tpu as pltpu

_CH = 4096
_W = 16
_P = 64
_REP = 8

_NT = (((1,), (1,)), ((), ()))
_NN = (((1,), (0,)), ((), ()))


def _dot(a, b, dims=_NN):
    return lax.dot_general(a, b, dims, preferred_element_type=jnp.float32)


def _bf(x):
    return x.astype(jnp.bfloat16).astype(jnp.float32)


def _layernorm(x, eps=1e-5):
    m = jnp.mean(x, axis=-1, keepdims=True)
    d = x - m
    v = jnp.mean(d * d, axis=-1, keepdims=True)
    return d / jnp.sqrt(v + eps)


def _rep_rows(x):
    b, n = x.shape
    return jnp.concatenate(
        [jnp.broadcast_to(x[i:i + 1], (_REP, n)) for i in range(b)], axis=0)


def _make_kernel(B, H, Sk, Dh, D, F, CH):
    NC = Sk // CH
    R = 2 * NC
    BH = B * H

    def kernel(x_hbm, c_hbm, wr_hbm, wmod_hbm, wq_hbm, k_hbm, v_hbm, woT_hbm, wg_hbm, wu_hbm,
               wdT_hbm, out_ref,
               x_v, c_v, wr_v, wmod_v, wq_v, woT_v, wg_v, wu_v, wdT_v,
               ring, q_s, s_s, acc_s, wsem, rsem):

        wcopy = [
            pltpu.make_async_copy(src, dst, wsem.at[i])
            for i, (src, dst) in enumerate([
                (c_hbm, c_v), (x_hbm, x_v), (wmod_hbm, wmod_v), (wq_hbm, wq_v),
                (woT_hbm, woT_v), (wr_hbm, wr_v), (wg_hbm, wg_v), (wu_hbm, wu_v),
                (wdT_hbm, wdT_v)])
        ]

        class stream:
            def __init__(self, bh, j):
                self.bh, self.j = bh, j

            def start(self):
                bh, j = self.bh, self.j
                src = k_hbm if j < NC else v_hbm
                S, L = Sk // _W, CH // _W
                for p in range(L // _P):
                    for w in range(_W):
                        pltpu.make_async_copy(
                            src.at[bh, pl.ds(w * S + (j % NC) * L + p * _P, _P), :],
                            ring.at[j, pl.ds(w * L + p * _P, _P), :],
                            rsem.at[j]).start(priority=w % 2)

            def wait(self):
                j = self.j
                pltpu.make_async_copy(ring.at[j], ring.at[j], rsem.at[j]).wait()

        for i in range(4):
            wcopy[i].start()
        for j in range(NC):
            stream(0, j).start()
        wcopy[4].start()
        for j in range(NC, R):
            stream(0, j).start()
        for i in range(5, 9):
            wcopy[i].start()

        wcopy[0].wait()
        wcopy[1].wait()
        cf = c_v[...].astype(jnp.float32)
        sc = _rep_rows(cf * jax.nn.sigmoid(cf)).astype(jnp.bfloat16)
        x = _rep_rows(x_v[...].astype(jnp.float32))
        ln1 = _bf(_layernorm(x))
        wcopy[2].wait()
        mod = _bf(_dot(sc, wmod_v[...]))
        h1 = _bf(_bf(ln1 * _bf(1.0 + mod[:, D:2 * D])) + mod[:, 0:D])
        wcopy[3].wait()
        q = _dot(h1.astype(jnp.bfloat16), wq_v[...]).astype(jnp.bfloat16)
        for b in range(B):
            for h in range(H):
                q_s[b * H + h] = q[b * _REP:(b + 1) * _REP, h * Dh:(h + 1) * Dh]
        acc_s[...] = jnp.zeros(acc_s.shape, jnp.float32)
        wcopy[4].wait()

        def bh_step(bh, carry):
            nxt = bh + 1
            qh = q_s[bh]
            mx = None
            for j in range(NC):
                stream(bh, j).wait()
                s = _dot(qh, ring[j], _NT) * (Dh ** -0.5)
                s_s[j] = s
                cm = s[:, 0:128]
                for t in range(1, CH // 128):
                    cm = jnp.maximum(cm, s[:, t * 128:(t + 1) * 128])
                mx = cm if mx is None else jnp.maximum(mx, cm)

                @pl.when(nxt < BH)
                def _():
                    stream(nxt, j).start()
            m = jnp.max(mx, axis=-1, keepdims=True)
            l = None
            o = None
            for j in range(NC, R):
                stream(bh, j).wait()
                p = jnp.exp(s_s[j - NC] - m)
                ps = p[:, 0:128]
                for t in range(1, CH // 128):
                    ps = ps + p[:, t * 128:(t + 1) * 128]
                l = ps if l is None else l + ps
                pv = _dot(p.astype(jnp.bfloat16), ring[j])
                o = pv if o is None else o + pv

                @pl.when(nxt < BH)
                def _():
                    stream(nxt, j).start()
            o = (o / jnp.sum(l, axis=-1, keepdims=True)).astype(jnp.bfloat16)
            b = bh // H
            h = bh - b * H
            wo_h = woT_v[:, pl.ds(pl.multiple_of(h * Dh, Dh), Dh)]
            acc_s[b] = acc_s[b] + _dot(o, wo_h, _NT)
            return carry

        lax.fori_loop(0, BH, bh_step, 0)

        attn = _bf(acc_s[...].reshape(B * _REP, D))
        x2 = _bf(x + _bf(mod[:, 2 * D:3 * D] * attn))
        ln2 = _bf(_layernorm(x2))
        h2 = _bf(_bf(ln2 * _bf(1.0 + mod[:, 4 * D:5 * D])) + mod[:, 3 * D:4 * D])
        h2b = h2.astype(jnp.bfloat16)
        for i in range(5, 9):
            wcopy[i].wait()
        r = _bf(jnp.sum(h2 * wr_v[...].astype(jnp.float32).reshape(1, D), axis=-1, keepdims=True))
        g = _bf(_dot(h2b, wg_v[...]))
        g = _bf(g * jax.nn.sigmoid(g))
        u = _bf(_dot(h2b, wu_v[...]))
        y = _bf(_dot((g * u).astype(jnp.bfloat16), wdT_v[...], _NT))
        y = _bf(y * _bf(jax.nn.sigmoid(r)))
        moe = _bf(h2 + (h2 * 0.0 + y))
        res = x2 + _bf(mod[:, 5 * D:6 * D] * moe)
        for b in range(B):
            out_ref[b:b + 1, :] = res[b * _REP:b * _REP + 1].astype(out_ref.dtype)

    return kernel, NC, R


@jax.jit
def pallas_adaLN_cond__mha_block_cached__moe_arch_mod__decode_kernel(
    A_x: jax.Array,
    A_k_cache: jax.Array,
    A_v_cache: jax.Array,
    A_wq: jax.Array,
    A_wo: jax.Array,
    B_x: jax.Array,
    B_w_r: jax.Array,
    B_w_gate: jax.Array,
    B_w_up: jax.Array,
    B_w_down: jax.Array,
    c: jax.Array,
    w_mod: jax.Array,
):
    del B_x
    B, Sq, D = A_x.shape
    _, H, Sk, Dh = A_k_cache.shape
    F = B_w_gate.shape[1]
    assert Sq == 1
    CH = _CH
    kernel, NC, R = _make_kernel(B, H, Sk, Dh, D, F, CH)
    bf = jnp.bfloat16
    hbm = pl.BlockSpec(memory_space=pltpu.HBM)

    out = pl.pallas_call(
        kernel,
        out_shape=jax.ShapeDtypeStruct((B, D), A_x.dtype),
        in_specs=[hbm] * 11,
        out_specs=pl.BlockSpec(memory_space=pltpu.VMEM),
        scratch_shapes=[
            pltpu.VMEM((B, D), bf), pltpu.VMEM((B, D), bf), pltpu.VMEM((D,), bf),
            pltpu.VMEM((D, 6 * D), bf), pltpu.VMEM((D, H * Dh), bf), pltpu.VMEM((D, H * Dh), bf),
            pltpu.VMEM((D, F), bf), pltpu.VMEM((D, F), bf), pltpu.VMEM((D, F), bf),
            pltpu.VMEM((R, CH, Dh), bf),
            pltpu.VMEM((B * H, _REP, Dh), bf),
            pltpu.VMEM((NC, _REP, CH), jnp.float32),
            pltpu.VMEM((B, _REP, D), jnp.float32),
            pltpu.SemaphoreType.DMA((9,)),
            pltpu.SemaphoreType.DMA((R,)),
        ],
        compiler_params=pltpu.CompilerParams(vmem_limit_bytes=100 * 1024 * 1024),
    )(
        A_x.reshape(B, D), c, B_w_r, w_mod, A_wq,
        A_k_cache.reshape(B * H, Sk, Dh), A_v_cache.reshape(B * H, Sk, Dh),
        A_wo.T, B_w_gate, B_w_up, B_w_down.T,
    )
    return out.reshape(B, Sq, D)
```
